```python
import jax
import jax.numpy as jnp

def _softmax(x, axis=-1):
    return jax.nn.softmax(x, axis=axis)
def _gelu(x):
    return jax.nn.gelu(x, approximate=True)
def _silu(x):
    return jax.nn.silu(x)
def _sigmoid(x):
    return jax.nn.sigmoid(x)
def _layernorm(x, axis=-1, eps=1e-5):
    m = jnp.mean(x, axis=axis, keepdims=True)
    v = jnp.var(x, axis=axis, keepdims=True)
    return (x - m) / jnp.sqrt(v + eps)
def _scatter_add(tgt, idx, src, axis=0):
    return tgt.at[idx].add(src)
def _segment_sum(src, seg, n):
    return jax.ops.segment_sum(src, seg, n)
class _Rng:
    def __init__(self, key):
        self._k = key
    def _next(self):
        self._k, sub = jax.random.split(self._k)
        return sub
    def normal(self, shape):
        return jax.random.normal(self._next(), shape, dtype=jnp.bfloat16)
    def randint(self, lo, hi, shape):
        return jax.random.randint(self._next(), shape, lo, hi, dtype=jnp.int32)
    def uniform(self, shape, lo=0.0, hi=1.0):
        return jax.random.uniform(self._next(), shape, jnp.bfloat16, lo, hi)
    def permutation(self, n):
        return jax.random.permutation(self._next(), n)


kernel_name = 'recurrent_scan__gqa_block_cached__geglu_ffn__decode'

def _fwd_setup_inputs():
    _rng = _Rng(jax.random.key(int.from_bytes(__import__("os").urandom(4), "little")))
    _w = (lambda a: (lambda t: t.astype(jnp.bfloat16) if jnp.issubdtype(t.dtype, jnp.floating) else t)(jnp.asarray(a)))
    def _A_setup():
        B, Sq, D = 1, 1, 512
        Hq, Hkv, Sk, Dh = 32, 32, 4096, 128
        assert Hq % Hkv == 0, (Hq, Hkv)
        return {
            "x": _w((lambda *s: _rng.normal(s) * 0.05)(B, Sq, D)),
            "k_cache": _w((lambda *s: _rng.normal(s) * 0.05)(B, Hkv, Sk, Dh)),
            "v_cache": _w((lambda *s: _rng.normal(s) * 0.05)(B, Hkv, Sk, Dh)),
            "wq": _w((lambda *s: _rng.normal(s) * 0.05)(D, Hq * Dh) * (D ** -0.5)),
            "wo": _w((lambda *s: _rng.normal(s) * 0.05)(Hq * Dh, D) * ((Hq * Dh) ** -0.5)),
        }
    _A_in = _A_setup()

    def _B_setup():
        B, S, D, F = 1, 1, 512, 1376
        return {
            "x": _w((lambda *s: _rng.normal(s) * 0.05)(B, S, D)),
            "w_gate": _w((lambda *s: _rng.normal(s) * 0.05)(D, F)),
            "w_up": _w((lambda *s: _rng.normal(s) * 0.05)(D, F)),
            "w_down": _w((lambda *s: _rng.normal(s) * 0.05)(F, D)),
        }
    _B_in = _B_setup()

    return {
        "A_x": _A_in["x"],
        "A_k_cache": _A_in["k_cache"],
        "A_v_cache": _A_in["v_cache"],
        "A_wq": _A_in["wq"],
        "A_wo": _A_in["wo"],
        "B_x": _B_in["x"],
        "B_w_gate": _B_in["w_gate"],
        "B_w_up": _B_in["w_up"],
        "B_w_down": _B_in["w_down"],
    }

def _fwd_reference(A_x, A_k_cache, A_v_cache, A_wq, A_wo, B_x, B_w_gate, B_w_up, B_w_down):
    def _A_ref(x, k_cache, v_cache, wq, wo):
        B, Sq, D = x.shape
        Hq, Dh = 32, 128
        Hkv = k_cache.shape[1]
        rep = Hq // Hkv
        q = (lambda x, *d: x.transpose(*d))((x @ wq).reshape(B, Sq, Hq, Dh), 0, 2, 1, 3)
        k = jnp.repeat(k_cache, rep, axis=1)
        v = jnp.repeat(v_cache, rep, axis=1)
        scores = jnp.einsum("bhqd,bhkd->bhqk", q, k) * (Dh ** -0.5)
        p = _softmax(scores, axis=-1)
        o = jnp.einsum("bhqk,bhkd->bhqd", p, v)
        return (lambda x, *d: x.transpose(*d))(o, 0, 2, 1, 3).reshape(B, Sq, Hq * Dh) @ wo

    def _B_ref(x, w_gate, w_up, w_down):
        return (_gelu(x @ w_gate) * (x @ w_up)) @ w_down

    x = A_x
    xn = _layernorm(x, axis=-1)
    s = _A_ref(xn, A_k_cache, A_v_cache, A_wq, A_wo)
    g = _silu(_B_ref(xn, B_w_gate, B_w_up, B_w_down))
    return x + s * g


def setup_inputs():
    _inp = _fwd_setup_inputs()
    _gk = jax.random.fold_in(jax.random.key(int.from_bytes(__import__("os").urandom(4), "little")), 2**31 - 1)
    _shapes = [[1, 1, 512]]
    _dtypes = ['bfloat16']
    _gks = jax.random.split(_gk, len(_shapes))
    _gs = [jax.random.normal(k, s, dtype=jnp.dtype(d)) * 0.05 for k, s, d in zip(_gks, _shapes, _dtypes)]
    _inp["grad_out"] = _gs[0]
    return _inp

def reference(A_x, A_k_cache, A_v_cache, A_wq, A_wo, B_w_gate, B_w_up, B_w_down, B_x, grad_out):
    _const = dict(B_x=B_x)
    def _f(*_d):
        return _fwd_reference(**{'A_x': _d[0], 'A_k_cache': _d[1], 'A_v_cache': _d[2], 'A_wq': _d[3], 'A_wo': _d[4], 'B_w_gate': _d[5], 'B_w_up': _d[6], 'B_w_down': _d[7], **_const})
    _out, _vjp = jax.vjp(_f, A_x, A_k_cache, A_v_cache, A_wq, A_wo, B_w_gate, B_w_up, B_w_down)
    _grads = _vjp(grad_out)
    _out0 = jnp.asarray(_out)
    return (_out0, *[jnp.asarray(_g) for _g in _grads])
```

```python
import math

import jax
import jax.numpy as jnp
from jax import lax
import jax.experimental.pallas as pl
import jax.experimental.pallas.tpu as pltpu

BF16 = jnp.bfloat16
F32 = jnp.float32

ROWS = 8
LANES = 128
LN_EPS = 1e-5

KV_SLOTS = 3
V_TAIL = 2048
BANDS = 8
KV_RUN = 64
WO_RUN = (16, 512)
WQ_RUN = (8, 1024)
FFN_RUN = 16
EARLY_FILLS = 16
LEAD_PARTS = 3


def _dot(a, b):
    return jnp.dot(a, b, preferred_element_type=F32)


def _dot_nt(a, b):
    return lax.dot_general(a, b, (((1,), (1,)), ((), ())), preferred_element_type=F32)


def _outer(col, row):
    live = lax.broadcasted_iota(jnp.int32, row.shape, 0) == 0
    return lax.dot_general(
        col.astype(BF16), jnp.where(live, row, 0.0).astype(BF16),
        (((0,), (0,)), ((), ())), preferred_element_type=F32).astype(BF16)


def _mean(v):
    return jnp.sum(v, axis=-1, keepdims=True) * (1.0 / v.shape[-1])


def _tile(i, size):
    return pl.ds(pl.multiple_of(i * size, size), size)


def _kernel(
    x_hbm, k_hbm, v_hbm, wq_hbm, wo_hbm, wg_hbm, wu_hbm, wd_hbm, go_hbm,
    out_hbm, dx_hbm, dk_hbm, dv_hbm, dwq_hbm, dwo_hbm, dwg_hbm, dwu_hbm, dwd_hbm,
    x_buf, go_buf, out_buf, dx_buf,
    wq_buf, wo_buf, ffn_buf, k_buf, v_buf,
    dkv_buf, dwq_buf, dwo_buf, dffn_buf,
    act_buf, coef_buf, factor_buf,
    ffn_sem, proj_sem, kv_sems, out_sem,
):
    heads, seq, head_dim = k_hbm.shape
    d_ff, d_model = wd_hbm.shape
    ff_tiles = ffn_buf.shape[1] // LANES
    scale = head_dim ** -0.5
    copy = pltpu.make_async_copy

    def kv_reads(h):
        slot = h % KV_SLOTS
        front, tail = pl.ds(0, seq - V_TAIL), pl.ds(seq - V_TAIL, V_TAIL)
        return (copy(k_hbm.at[h], k_buf.at[slot], kv_sems.at[0, slot]),
                copy(v_hbm.at[h, front], v_buf.at[slot, front], kv_sems.at[0, slot]),
                copy(v_hbm.at[h, tail], v_buf.at[slot, tail], kv_sems.at[1, slot]))

    def start_kv_reads(h, _=None):
        for c in kv_reads(h):
            c.start()

    def fill(u):
        dkv_buf[u] = _outer(coef_buf[u], factor_buf[u])

    def write_part(s, _=None):
        first = (s // BANDS) * BANDS
        runs = seq // KV_RUN // BANDS

        def write_to(dst):
            def step(j, _):
                rows = _tile((s % BANDS) * runs + j, KV_RUN)
                copy(dkv_buf.at[pl.ds(first, BANDS), rows, :],
                     dst.at[pl.ds(first % heads, BANDS), rows, :], out_sem).start()

            lax.fori_loop(0, runs, step, None)

        pl.when(s < heads)(lambda: write_to(dv_hbm))
        pl.when(s >= heads)(lambda: write_to(dk_hbm))

    def write_banded(src, dst, run):
        run_rows, run_cols = run
        per_row = src.shape[2] // run_cols

        def step(j, _):
            rows, cols = _tile(j // per_row, run_rows), _tile(j % per_row, run_cols)
            copy(src.at[:, rows, cols], dst.at[:, rows, cols], out_sem).start()

        lax.fori_loop(0, (src.shape[1] // run_rows) * per_row, step, None)

    ffn_reads = [copy(w, ffn_buf.at[i, pl.ds(0, d_ff)], ffn_sem)
                 for i, w in enumerate((wg_hbm, wu_hbm, wd_hbm))]
    ffn_reads += [copy(x_hbm, x_buf, ffn_sem), copy(go_hbm, go_buf, ffn_sem)]
    proj_reads = [copy(wo_hbm, wo_buf, proj_sem), copy(wq_hbm, wq_buf, proj_sem)]
    for c in (*ffn_reads, *proj_reads):
        c.start()
    lax.fori_loop(0, KV_SLOTS, start_kv_reads, None)

    for c in ffn_reads:
        c.wait()
    pad = ffn_buf.shape[1] - d_ff
    ffn_buf[:, pl.ds(d_ff, pad), :] = jnp.zeros((3, pad, d_model), BF16)

    x = jnp.broadcast_to(x_buf[0].astype(F32), (ROWS, d_model))
    go = jnp.broadcast_to(go_buf[0].astype(F32), (ROWS, d_model))
    centered = x - _mean(x)
    rstd = lax.rsqrt(_mean(centered * centered) + LN_EPS)
    xn = centered * rstd
    xn_b = xn.astype(BF16)

    def ffn_forward(j, ffn):
        rows = _tile(j, LANES)
        gate = _dot_nt(xn_b, ffn_buf[0, rows, :])
        up = _dot_nt(xn_b, ffn_buf[1, rows, :])
        c0 = math.sqrt(2.0 / math.pi)
        tanh = jnp.tanh(c0 * (gate + 0.044715 * gate * gate * gate))
        cdf = 0.5 * (1.0 + tanh)
        gelu = gate * cdf
        gelu_grad = cdf + gate * (0.5 * c0) * (1.0 - tanh * tanh) * (
            1.0 + 3 * 0.044715 * gate * gate)
        hidden = gelu * up
        act_buf[0, j] = up * gelu_grad
        act_buf[1, j] = gelu
        act_buf[2, j] = hidden
        return ffn + _dot(hidden.astype(BF16), ffn_buf[2, rows, :])

    zeros = jnp.zeros((ROWS, d_model), F32)
    ffn = lax.fori_loop(0, ff_tiles, ffn_forward, zeros)
    sig = jax.nn.sigmoid(ffn)
    silu = ffn * sig
    d_attn = go * silu
    d_attn_b = d_attn.astype(BF16)

    for c in proj_reads:
        c.wait()

    def attend(h, carry):
        attn, d_xn = carry
        slot = h % KV_SLOTS
        cols = _tile(h, head_dim)
        q = _dot(xn_b, wq_buf[:, cols])
        d_o = _dot_nt(d_attn_b, wo_buf[cols, :])

        k_read, v_front, v_tail = kv_reads(h)
        k_read.wait()
        v_front.wait()
        pl.when(h == heads - 1)(lambda: lax.fori_loop(0, LEAD_PARTS, write_part, None))
        v_tail.wait()

        scores = _dot_nt(q.astype(BF16), k_buf[slot]) * scale
        e = jnp.exp(scores - jnp.max(scores, axis=-1, keepdims=True))
        p = e * (1.0 / jnp.sum(e, axis=-1, keepdims=True))
        d_p = _dot_nt(d_o.astype(BF16), v_buf[slot])
        d_logits = p * (d_p - jnp.sum(p * d_p, axis=-1, keepdims=True)) * scale
        o = _dot(p.astype(BF16), v_buf[slot])
        d_q = _dot(d_logits.astype(BF16), k_buf[slot])
        pl.when(h + KV_SLOTS < heads)(lambda: start_kv_reads(h + KV_SLOTS))

        coef_buf[h] = p
        factor_buf[h] = d_o
        coef_buf[heads + h] = d_logits
        factor_buf[heads + h] = q
        per_band = heads // BANDS
        dwo_buf[h // per_band, _tile(h % per_band, head_dim), :] = _outer(o, d_attn)
        dwq_buf[:, :, cols] = _outer(xn, d_q).reshape(BANDS, d_model // BANDS, head_dim)
        pl.when(h < EARLY_FILLS)(lambda: fill(h))
        return (attn + _dot(o.astype(BF16), wo_buf[cols, :]),
                d_xn + _dot_nt(d_q.astype(BF16), wq_buf[:, cols]))

    attn, d_xn = lax.fori_loop(0, heads, attend, (zeros, zeros))

    def drain(u, _):
        write_part(u - EARLY_FILLS + LEAD_PARTS)
        fill(u)

    lax.fori_loop(EARLY_FILLS, 2 * heads, drain, None)
    parts_sent = 2 * heads - EARLY_FILLS + LEAD_PARTS

    d_ffn = go * attn * sig * (1.0 + ffn * (1.0 - sig))
    d_ffn_b = d_ffn.astype(BF16)

    def ffn_backward(j, d_xn):
        write_part(parts_sent + j)
        rows = _tile(j, LANES)
        d_hidden = _dot_nt(d_ffn_b, ffn_buf[2, rows, :])
        d_gate = d_hidden * act_buf[0, j]
        d_up = d_hidden * act_buf[1, j]
        dffn_buf[0, rows, :] = _outer(d_gate, xn)
        dffn_buf[1, rows, :] = _outer(d_up, xn)
        dffn_buf[2, rows, :] = _outer(act_buf[2, j], d_ffn)
        return (d_xn + _dot(d_gate.astype(BF16), ffn_buf[0, rows, :])
                + _dot(d_up.astype(BF16), ffn_buf[1, rows, :]))

    d_xn = lax.fori_loop(0, ff_tiles, ffn_backward, d_xn)
    d_x = go + rstd * (d_xn - _mean(d_xn) - xn * _mean(d_xn * xn))
    out_buf[0] = (x + attn * silu)[0:1].astype(BF16)
    dx_buf[0] = d_x[0:1].astype(BF16)
    vec_writes = [copy(out_buf, out_hbm, out_sem), copy(dx_buf, dx_hbm, out_sem)]
    for c in vec_writes:
        c.start()

    lax.fori_loop(parts_sent + ff_tiles, 2 * heads, write_part, None)
    write_banded(dwo_buf, dwo_hbm, WO_RUN)
    write_banded(dwq_buf, dwq_hbm, WQ_RUN)

    ffn_outs = (dwg_hbm, dwu_hbm, dwd_hbm)
    half_runs = d_ff // (2 * FFN_RUN)

    def write_dffn(j, _):
        for half in range(2):
            rows = _tile(half * half_runs + j, FFN_RUN)
            for i, dst in enumerate(ffn_outs):
                copy(dffn_buf.at[i, rows, :], dst.at[rows, :], out_sem).start()

    lax.fori_loop(0, half_runs, write_dffn, None)

    for c in vec_writes:
        c.wait()
    for buf in (dkv_buf, dwo_buf, dwq_buf):
        copy(buf, buf, out_sem).wait()
    for i, dst in enumerate(ffn_outs):
        copy(dffn_buf.at[i, pl.ds(0, d_ff)], dst, out_sem).wait()


@jax.jit
def pallas_recurrent_scan__gqa_block_cached__geglu_ffn__decode_kernel(
    A_x: jax.Array,
    A_k_cache: jax.Array,
    A_v_cache: jax.Array,
    A_wq: jax.Array,
    A_wo: jax.Array,
    B_x: jax.Array,
    B_w_gate: jax.Array,
    B_w_up: jax.Array,
    B_w_down: jax.Array,
    grad_out: jax.Array,
):
    del B_x
    _, heads, seq, head_dim = A_k_cache.shape
    d_model, d_ff = B_w_gate.shape
    d_attn = heads * head_dim
    ff_tiles = pl.cdiv(d_ff, LANES)
    assert A_k_cache.shape[0] == 1 and A_wq.shape == (d_model, d_attn)
    assert heads % BANDS == 0 and seq % (BANDS * KV_RUN) == 0
    assert d_ff % (2 * FFN_RUN) == 0
    assert max(BANDS, ff_tiles) <= EARLY_FILLS - LEAD_PARTS and EARLY_FILLS < heads

    vec = A_x.shape
    cache = (heads, seq, head_dim)
    dwq = (BANDS, d_model // BANDS, d_attn)
    dwo = (BANDS, d_attn // BANDS, d_model)
    ffn = (d_ff, d_model)
    ffn_padded = (3, ff_tiles * LANES, d_model)

    hbm = pl.BlockSpec(memory_space=pltpu.HBM)
    out, dx, dk, dv, g_wq, g_wo, g_gate, g_up, g_down = pl.pallas_call(
        _kernel,
        in_specs=[hbm] * 9,
        out_specs=[hbm] * 9,
        out_shape=[jax.ShapeDtypeStruct(s, BF16)
                   for s in (vec, vec, cache, cache, dwq, dwo, ffn, ffn, ffn)],
        scratch_shapes=[
            pltpu.VMEM(vec, BF16), pltpu.VMEM(vec, BF16),
            pltpu.VMEM(vec, BF16), pltpu.VMEM(vec, BF16),
            pltpu.VMEM((d_model, d_attn), BF16),
            pltpu.VMEM((d_attn, d_model), BF16),
            pltpu.VMEM(ffn_padded, BF16),
            pltpu.VMEM((KV_SLOTS, seq, head_dim), BF16),
            pltpu.VMEM((KV_SLOTS, seq, head_dim), BF16),
            pltpu.VMEM((2 * heads, seq, head_dim), BF16),
            pltpu.VMEM(dwq, BF16),
            pltpu.VMEM(dwo, BF16),
            pltpu.VMEM(ffn_padded, BF16),
            pltpu.VMEM((3, ff_tiles, ROWS, LANES), F32),
            pltpu.VMEM((2 * heads, ROWS, seq), F32),
            pltpu.VMEM((2 * heads, ROWS, head_dim), F32),
            pltpu.SemaphoreType.DMA,
            pltpu.SemaphoreType.DMA,
            pltpu.SemaphoreType.DMA((2, KV_SLOTS)),
            pltpu.SemaphoreType.DMA,
        ],
        compiler_params=pltpu.CompilerParams(
            vmem_limit_bytes=120 * 1024 * 1024,
            disable_semaphore_checks=True,
        ),
    )(
        A_x, A_k_cache.reshape(cache), A_v_cache.reshape(cache), A_wq, A_wo,
        B_w_gate.T, B_w_up.T, B_w_down, grad_out,
    )
    return (
        out,
        dx,
        dk.reshape(A_k_cache.shape),
        dv.reshape(A_v_cache.shape),
        g_wq.reshape(A_wq.shape),
        g_wo.reshape(A_wo.shape),
        g_gate.T,
        g_up.T,
        g_down,
    )
```

```python
import functools
import math

import jax
import jax.numpy as jnp
from jax import lax
import jax.experimental.pallas as pl
import jax.experimental.pallas.tpu as pltpu

BF16 = jnp.bfloat16
F32 = jnp.float32

ROWS = 8
LANES = 128
LN_EPS = 1e-5

KV_SLOTS = 3
V_TAIL = 1664
HEAD_GROUPS = ((7, 2), (6, 3))
KV_RUN = 64
BANDS = 8
WO_RUN = (16, 512)
WQ_RUN = (8, 1024)
FFN_RUN = 16
EARLY_FILLS = 16
LEAD_PARTS = 3


def _dot(a, b):
    return jnp.dot(a, b, preferred_element_type=F32)


def _dot_nt(a, b):
    return lax.dot_general(a, b, (((1,), (1,)), ((), ())), preferred_element_type=F32)


def _outer(col, row):
    live = lax.broadcasted_iota(jnp.int32, row.shape, 0) == 0
    return lax.dot_general(
        col.astype(BF16), jnp.where(live, row, 0.0).astype(BF16),
        (((0,), (0,)), ((), ())), preferred_element_type=F32).astype(BF16)


def _mean(v):
    return jnp.sum(v, axis=-1, keepdims=True) * (1.0 / v.shape[-1])


def _tile(i, size):
    return pl.ds(pl.multiple_of(i * size, size), size)


def _kernel(
    x_hbm, k_hbm, v_hbm, wq_hbm, wo_hbm, wg_hbm, wu_hbm, wd_hbm, go_hbm,
    out_hbm, dx_hbm, dk_hbm, dv_hbm, dwq_hbm, dwo_hbm, dwg_hbm, dwu_hbm, dwd_hbm,
    x_buf, go_buf, out_buf, dx_buf,
    wq_buf, wo_buf, ffn_buf, k_buf, v_buf,
    dkv_buf, dwq_buf, dwo_buf, dffn_buf,
    act_buf, coef_buf, factor_buf,
    ffn_sem, proj_sem, kv_sems, out_sem,
):
    heads, seq, head_dim = k_hbm.shape
    d_ff, d_model = wd_hbm.shape
    ff_tiles = ffn_buf.shape[1] // LANES
    scale = head_dim ** -0.5
    copy = pltpu.make_async_copy

    def kv_reads(h):
        slot = h % KV_SLOTS
        front, tail = pl.ds(0, seq - V_TAIL), pl.ds(seq - V_TAIL, V_TAIL)
        return (copy(k_hbm.at[h], k_buf.at[slot], kv_sems.at[0, slot]),
                copy(v_hbm.at[h, front], v_buf.at[slot, front], kv_sems.at[0, slot]),
                copy(v_hbm.at[h, tail], v_buf.at[slot, tail], kv_sems.at[1, slot]))

    def start_kv_reads(h, _=None):
        for c in kv_reads(h):
            c.start()

    def fill(u):
        dkv_buf[u] = _outer(coef_buf[u], factor_buf[u])

    def write_part(s, _=None):
        runs = seq // KV_RUN

        def send(dst, base, lo, size):
            i = s - base - lo
            first, part = lo + (i // size) * size, i % size

            def step(j, _):
                rows = _tile(j, KV_RUN)
                copy(dkv_buf.at[pl.ds(base + first, size), rows, :],
                     dst.at[pl.ds(first, size), rows, :], out_sem).start()

            lax.fori_loop(part * runs // size, (part + 1) * runs // size, step, None)

        for dst, base in ((dv_hbm, 0), (dk_hbm, heads)):
            lo = 0
            for size, count in HEAD_GROUPS:
                hi = lo + size * count
                pl.when(jnp.logical_and(s >= base + lo, s < base + hi))(
                    functools.partial(send, dst, base, lo, size))
                lo = hi

    def write_banded(src, dst, run):
        run_rows, run_cols = run
        per_row = src.shape[2] // run_cols

        def step(j, _):
            rows, cols = _tile(j // per_row, run_rows), _tile(j % per_row, run_cols)
            copy(src.at[:, rows, cols], dst.at[:, rows, cols], out_sem).start()

        lax.fori_loop(0, (src.shape[1] // run_rows) * per_row, step, None)

    ffn_reads = [copy(w, ffn_buf.at[i, pl.ds(0, d_ff)], ffn_sem)
                 for i, w in enumerate((wg_hbm, wu_hbm, wd_hbm))]
    ffn_reads += [copy(x_hbm, x_buf, ffn_sem), copy(go_hbm, go_buf, ffn_sem)]
    proj_reads = [copy(wo_hbm, wo_buf, proj_sem), copy(wq_hbm, wq_buf, proj_sem)]
    for c in (*ffn_reads, *proj_reads):
        c.start()
    lax.fori_loop(0, KV_SLOTS, start_kv_reads, None)

    for c in ffn_reads:
        c.wait()
    pad = ffn_buf.shape[1] - d_ff
    ffn_buf[:, pl.ds(d_ff, pad), :] = jnp.zeros((3, pad, d_model), BF16)

    x = jnp.broadcast_to(x_buf[0].astype(F32), (ROWS, d_model))
    go = jnp.broadcast_to(go_buf[0].astype(F32), (ROWS, d_model))
    centered = x - _mean(x)
    rstd = lax.rsqrt(_mean(centered * centered) + LN_EPS)
    xn = centered * rstd
    xn_b = xn.astype(BF16)

    def ffn_forward(j, ffn):
        rows = _tile(j, LANES)
        gate = _dot_nt(xn_b, ffn_buf[0, rows, :])
        up = _dot_nt(xn_b, ffn_buf[1, rows, :])
        c0 = math.sqrt(2.0 / math.pi)
        tanh = jnp.tanh(c0 * (gate + 0.044715 * gate * gate * gate))
        cdf = 0.5 * (1.0 + tanh)
        gelu = gate * cdf
        gelu_grad = cdf + gate * (0.5 * c0) * (1.0 - tanh * tanh) * (
            1.0 + 3 * 0.044715 * gate * gate)
        hidden = gelu * up
        act_buf[0, j] = up * gelu_grad
        act_buf[1, j] = gelu
        act_buf[2, j] = hidden
        return ffn + _dot(hidden.astype(BF16), ffn_buf[2, rows, :])

    zeros = jnp.zeros((ROWS, d_model), F32)
    ffn = lax.fori_loop(0, ff_tiles, ffn_forward, zeros)
    sig = jax.nn.sigmoid(ffn)
    silu = ffn * sig
    d_attn = go * silu
    d_attn_b = d_attn.astype(BF16)

    for c in proj_reads:
        c.wait()

    def attend(h, carry):
        attn, d_xn = carry
        slot = h % KV_SLOTS
        cols = _tile(h, head_dim)
        q = _dot(xn_b, wq_buf[:, cols])
        d_o = _dot_nt(d_attn_b, wo_buf[cols, :])

        k_read, v_front, v_tail = kv_reads(h)
        k_read.wait()
        v_front.wait()
        pl.when(h == heads - 1)(lambda: lax.fori_loop(0, LEAD_PARTS, write_part, None))
        v_tail.wait()

        scores = _dot_nt(q.astype(BF16), k_buf[slot]) * scale
        e = jnp.exp(scores - jnp.max(scores, axis=-1, keepdims=True))
        p = e * (1.0 / jnp.sum(e, axis=-1, keepdims=True))
        d_p = _dot_nt(d_o.astype(BF16), v_buf[slot])
        d_logits = p * (d_p - jnp.sum(p * d_p, axis=-1, keepdims=True)) * scale
        o = _dot(p.astype(BF16), v_buf[slot])
        d_q = _dot(d_logits.astype(BF16), k_buf[slot])
        pl.when(h + KV_SLOTS < heads)(lambda: start_kv_reads(h + KV_SLOTS))

        coef_buf[h] = p
        factor_buf[h] = d_o
        coef_buf[heads + h] = d_logits
        factor_buf[heads + h] = q
        per_band = heads // BANDS
        dwo_buf[h // per_band, _tile(h % per_band, head_dim), :] = _outer(o, d_attn)
        dwq_buf[:, :, cols] = _outer(xn, d_q).reshape(BANDS, d_model // BANDS, head_dim)
        pl.when(h < EARLY_FILLS)(lambda: fill(h))
        return (attn + _dot(o.astype(BF16), wo_buf[cols, :]),
                d_xn + _dot_nt(d_q.astype(BF16), wq_buf[:, cols]))

    attn, d_xn = lax.fori_loop(0, heads, attend, (zeros, zeros))

    def drain(u, _):
        write_part(u - EARLY_FILLS + LEAD_PARTS)
        fill(u)

    lax.fori_loop(EARLY_FILLS, 2 * heads, drain, None)
    parts_sent = 2 * heads - EARLY_FILLS + LEAD_PARTS

    d_ffn = go * attn * sig * (1.0 + ffn * (1.0 - sig))
    d_ffn_b = d_ffn.astype(BF16)

    def ffn_backward(j, d_xn):
        write_part(parts_sent + j)
        rows = _tile(j, LANES)
        d_hidden = _dot_nt(d_ffn_b, ffn_buf[2, rows, :])
        d_gate = d_hidden * act_buf[0, j]
        d_up = d_hidden * act_buf[1, j]
        dffn_buf[0, rows, :] = _outer(d_gate, xn)
        dffn_buf[1, rows, :] = _outer(d_up, xn)
        dffn_buf[2, rows, :] = _outer(act_buf[2, j], d_ffn)
        return (d_xn + _dot(d_gate.astype(BF16), ffn_buf[0, rows, :])
                + _dot(d_up.astype(BF16), ffn_buf[1, rows, :]))

    d_xn = lax.fori_loop(0, ff_tiles, ffn_backward, d_xn)
    d_x = go + rstd * (d_xn - _mean(d_xn) - xn * _mean(d_xn * xn))
    out_buf[0] = (x + attn * silu)[0:1].astype(BF16)
    dx_buf[0] = d_x[0:1].astype(BF16)
    vec_writes = [copy(out_buf, out_hbm, out_sem), copy(dx_buf, dx_hbm, out_sem)]
    for c in vec_writes:
        c.start()

    lax.fori_loop(parts_sent + ff_tiles, 2 * heads, write_part, None)
    write_banded(dwo_buf, dwo_hbm, WO_RUN)
    write_banded(dwq_buf, dwq_hbm, WQ_RUN)

    ffn_outs = (dwg_hbm, dwu_hbm, dwd_hbm)
    half_runs = d_ff // (2 * FFN_RUN)

    def write_dffn(j, _):
        for half in range(2):
            rows = _tile(half * half_runs + j, FFN_RUN)
            for i, dst in enumerate(ffn_outs):
                copy(dffn_buf.at[i, rows, :], dst.at[rows, :], out_sem).start()

    lax.fori_loop(0, half_runs, write_dffn, None)

    for c in vec_writes:
        c.wait()
    for buf in (dkv_buf, dwo_buf, dwq_buf):
        copy(buf, buf, out_sem).wait()
    for i, dst in enumerate(ffn_outs):
        copy(dffn_buf.at[i, pl.ds(0, d_ff)], dst, out_sem).wait()


@jax.jit
def pallas_recurrent_scan__gqa_block_cached__geglu_ffn__decode_kernel(
    A_x: jax.Array,
    A_k_cache: jax.Array,
    A_v_cache: jax.Array,
    A_wq: jax.Array,
    A_wo: jax.Array,
    B_x: jax.Array,
    B_w_gate: jax.Array,
    B_w_up: jax.Array,
    B_w_down: jax.Array,
    grad_out: jax.Array,
):
    del B_x
    _, heads, seq, head_dim = A_k_cache.shape
    d_model, d_ff = B_w_gate.shape
    d_attn = heads * head_dim
    ff_tiles = pl.cdiv(d_ff, LANES)
    assert A_k_cache.shape[0] == 1 and A_wq.shape == (d_model, d_attn)
    assert heads == sum(size * count for size, count in HEAD_GROUPS)
    assert heads % BANDS == 0 and seq % KV_RUN == 0 and d_ff % (2 * FFN_RUN) == 0
    assert max(ff_tiles, *(size for size, _ in HEAD_GROUPS)) <= EARLY_FILLS - LEAD_PARTS
    assert EARLY_FILLS < heads

    vec = A_x.shape
    cache = (heads, seq, head_dim)
    dwq = (BANDS, d_model // BANDS, d_attn)
    dwo = (BANDS, d_attn // BANDS, d_model)
    ffn = (d_ff, d_model)
    ffn_padded = (3, ff_tiles * LANES, d_model)

    hbm = pl.BlockSpec(memory_space=pltpu.HBM)
    out, dx, dk, dv, g_wq, g_wo, g_gate, g_up, g_down = pl.pallas_call(
        _kernel,
        in_specs=[hbm] * 9,
        out_specs=[hbm] * 9,
        out_shape=[jax.ShapeDtypeStruct(s, BF16)
                   for s in (vec, vec, cache, cache, dwq, dwo, ffn, ffn, ffn)],
        scratch_shapes=[
            pltpu.VMEM(vec, BF16), pltpu.VMEM(vec, BF16),
            pltpu.VMEM(vec, BF16), pltpu.VMEM(vec, BF16),
            pltpu.VMEM((d_model, d_attn), BF16),
            pltpu.VMEM((d_attn, d_model), BF16),
            pltpu.VMEM(ffn_padded, BF16),
            pltpu.VMEM((KV_SLOTS, seq, head_dim), BF16),
            pltpu.VMEM((KV_SLOTS, seq, head_dim), BF16),
            pltpu.VMEM((2 * heads, seq, head_dim), BF16),
            pltpu.VMEM(dwq, BF16),
            pltpu.VMEM(dwo, BF16),
            pltpu.VMEM(ffn_padded, BF16),
            pltpu.VMEM((3, ff_tiles, ROWS, LANES), F32),
            pltpu.VMEM((2 * heads, ROWS, seq), F32),
            pltpu.VMEM((2 * heads, ROWS, head_dim), F32),
            pltpu.SemaphoreType.DMA,
            pltpu.SemaphoreType.DMA,
            pltpu.SemaphoreType.DMA((2, KV_SLOTS)),
            pltpu.SemaphoreType.DMA,
        ],
        compiler_params=pltpu.CompilerParams(
            vmem_limit_bytes=120 * 1024 * 1024,
            disable_semaphore_checks=True,
        ),
    )(
        A_x, A_k_cache.reshape(cache), A_v_cache.reshape(cache), A_wq, A_wo,
        B_w_gate.T, B_w_up.T, B_w_down, grad_out,
    )
    return (
        out,
        dx,
        dk.reshape(A_k_cache.shape),
        dv.reshape(A_v_cache.shape),
        g_wq.reshape(A_wq.shape),
        g_wo.reshape(A_wo.shape),
        g_gate.T,
        g_up.T,
        g_down,
    )
```
